```python
import os as _os
_os.environ.setdefault('JAX_PLATFORMS', 'cpu')
import jax
import jax.numpy as jnp

def _softmax(x, axis=-1):
    return jax.nn.softmax(x, axis=axis)

def _gelu(x):
    return jax.nn.gelu(x, approximate=True)

def _silu(x):
    return jax.nn.silu(x)

def _sigmoid(x):
    return jax.nn.sigmoid(x)

def _layernorm(x, axis=-1, eps=1e-05):
    m = jnp.mean(x, axis=axis, keepdims=True)
    v = jnp.var(x, axis=axis, keepdims=True)
    return (x - m) / jnp.sqrt(v + eps)

def _scatter_add(tgt, idx, src, axis=0):
    return tgt.at[idx].add(src)

def _segment_sum(src, seg, n):
    return jax.ops.segment_sum(src, seg, n)

class _Rng:

    def __init__(self, key):
        self._k = key

    def _next(self):
        self._k, sub = jax.random.split(self._k)
        return sub

    def normal(self, shape):
        return jax.random.normal(self._next(), shape, dtype=jnp.bfloat16)

    def randint(self, lo, hi, shape):
        return jax.random.randint(self._next(), shape, lo, hi, dtype=jnp.int32)

    def uniform(self, shape, lo=0.0, hi=1.0):
        return jax.random.uniform(self._next(), shape, jnp.bfloat16, lo, hi)

    def permutation(self, n):
        return jax.random.permutation(self._next(), n)
kernel_name = 'standalone__conformer_conv_module__speech'

def setup_inputs():
    _rng = _Rng(jax.random.key(int.from_bytes(__import__("os").urandom(4), "little")))
    _w = lambda a: (lambda t: t.astype(jnp.bfloat16) if jnp.issubdtype(t.dtype, jnp.floating) else t)(jnp.asarray(a))
    B, T, D, K = (2, 16000, 256, 5)
    return {'x': _w((lambda *s: _rng.normal(s) * 0.2)(B, T, D)), 'w_pw1': _w((lambda *s: _rng.normal(s) * 0.2)(D, 2 * D)), 'dw': _w((lambda *s: _rng.normal(s) * 0.05)(K, D)), 'w_pw2': _w((lambda *s: _rng.normal(s) * 0.05)(D, D))}

def reference(x, w_pw1, dw, w_pw2):
    B, T, D = x.shape
    K = dw.shape[0]
    h = x @ w_pw1
    a, b = (h[..., :D].copy(), h[..., D:].copy())
    h = a * _sigmoid(b)
    pad = K // 2
    hp = jnp.pad(h, ((0, 0), (pad, pad), (0, 0)))
    out = jnp.zeros_like(h)
    for i in range(K):
        out = out + hp[:, i:i + T, :] * dw[i][None, None, :]
    return _silu(out) @ w_pw2
```

```python
import jax
import jax.numpy as jnp
import jax.experimental.pallas as pl
import jax.experimental.pallas.tpu as pltpu

TB = 1000 * 2
HALO = 16

@jax.jit
def pallas_standalone__conformer_conv_module__speech_kernel(x, w_pw1, dw, w_pw2):
    B, T, D = x.shape
    K = dw.shape[0]
    pad = K // 2
    nt = T // TB
    nh = T // HALO
    r = TB // HALO

    def kernel(x_ref, xp_ref, xn_ref, w1_ref, dw_ref, w2_ref, o_ref, g_scr):
        t = pl.program_id(1)

        def glu(xv):
            h = jnp.dot(xv, w1_ref[...], preferred_element_type=jnp.float32)
            return h[:, :D] * jax.nn.sigmoid(h[:, D:])

        g_scr[8:8 + TB, :] = glu(x_ref[0])
        gp = glu(xp_ref[0])
        gn = glu(xn_ref[0])
        g_scr[0:8, :] = jnp.where(t > 0, gp[8:16], 0.0)
        g_scr[8 + TB:16 + TB, :] = jnp.where(t < nt - 1, gn[0:8], 0.0)
        dwv = dw_ref[...].astype(jnp.float32)
        acc = g_scr[8 - pad:8 - pad + TB, :] * dwv[0:1, :]
        for k in range(1, K):
            acc = acc + g_scr[8 - pad + k:8 - pad + k + TB, :] * dwv[k:k + 1, :]
        s = (acc * jax.nn.sigmoid(acc)).astype(jnp.bfloat16)
        o_ref[0] = jnp.dot(s, w2_ref[...], preferred_element_type=jnp.float32).astype(o_ref.dtype)

    return pl.pallas_call(
        kernel,
        grid=(B, nt),
        in_specs=[
            pl.BlockSpec((1, TB, D), lambda b, t: (b, t, 0)),
            pl.BlockSpec((1, HALO, D), lambda b, t: (b, jnp.maximum(t * r - 1, 0), 0)),
            pl.BlockSpec((1, HALO, D), lambda b, t: (b, jnp.minimum((t + 1) * r, nh - 1), 0)),
            pl.BlockSpec((D, 2 * D), lambda b, t: (0, 0)),
            pl.BlockSpec((K, D), lambda b, t: (0, 0)),
            pl.BlockSpec((D, D), lambda b, t: (0, 0)),
        ],
        out_specs=pl.BlockSpec((1, TB, D), lambda b, t: (b, t, 0)),
        out_shape=jax.ShapeDtypeStruct((B, T, D), x.dtype),
        scratch_shapes=[pltpu.VMEM((TB + 16, D), jnp.float32)],
        compiler_params=pltpu.CompilerParams(
            dimension_semantics=("parallel", "arbitrary"),
            vmem_limit_bytes=100 * 1024 * 1024,
        ),
    )(x, x, x, w_pw1, dw, w_pw2)
```

```python
import jax
import jax.numpy as jnp
import jax.experimental.pallas as pl
import jax.experimental.pallas.tpu as pltpu

TB = 2000
CH = 80
HALO = 16

@jax.jit
def pallas_standalone__conformer_conv_module__speech_kernel(x, w_pw1, dw, w_pw2):
    B, T, D = x.shape
    K = dw.shape[0]
    pad = K // 2
    nt = T // TB
    nh = T // HALO
    r = TB // HALO
    L = CH // 8
    NC = TB // CH
    NL = D // 128

    def kernel(x_ref, xp_ref, xn_ref, w1_ref, dw_ref, w2_ref, o_ref, g_scr, s_scr, w1h_scr):
        b = pl.program_id(0)
        t = pl.program_id(1)

        @pl.when(jnp.logical_and(b == 0, t == 0))
        def _():
            w1h_scr[...] = w1_ref[...] * jnp.asarray(0.5, jnp.bfloat16)

        xcat = jnp.concatenate([xp_ref[0], x_ref[0], xn_ref[0]], axis=0)
        h = jnp.dot(xcat, w1h_scr[...], preferred_element_type=jnp.float32)
        a = h[:, :D]
        g = a + a * jnp.tanh(h[:, D:])
        dwv = dw_ref[...].astype(jnp.float32) * 0.5
        o = HALO - pad
        for c in range(NL):
            gc = g[:, c * 128:(c + 1) * 128]
            g_scr[c] = gc
            g_scr[c, 8:16, :] = jnp.where(t > 0, gc[8:16], 0.0)
            g_scr[c, 16 + TB:24 + TB, :] = jnp.where(t < nt - 1, gc[16 + TB:24 + TB], 0.0)
        wb = [[jnp.broadcast_to(dwv[k:k + 1, c * 128:(c + 1) * 128], (8, 128)) for k in range(K)] for c in range(NL)]
        for q in range(NC):
            for c in range(NL):
                def load(i):
                    return g_scr[c, pl.ds(q * CH + o + i, 8, stride=L), :]

                win = [load(i) for i in range(K - 1)]
                for j in range(L):
                    win.append(load(j + K - 1))
                    acc = win[0] * wb[c][0]
                    for k in range(1, K):
                        acc = acc + win[k] * wb[c][k]
                    s_scr[c, pl.ds(q * CH + j, 8, stride=L), :] = acc + acc * jnp.tanh(acc)
                    win.pop(0)
        s = jnp.concatenate([s_scr[c] for c in range(NL)], axis=1).astype(jnp.bfloat16)
        o_ref[0] = jnp.dot(s, w2_ref[...], preferred_element_type=jnp.float32).astype(o_ref.dtype)

    return pl.pallas_call(
        kernel,
        grid=(B, nt),
        in_specs=[
            pl.BlockSpec((1, TB, D), lambda b, t: (b, t, 0)),
            pl.BlockSpec((1, HALO, D), lambda b, t: (b, jnp.maximum(t * r - 1, 0), 0)),
            pl.BlockSpec((1, HALO, D), lambda b, t: (b, jnp.minimum((t + 1) * r, nh - 1), 0)),
            pl.BlockSpec((D, 2 * D), lambda b, t: (0, 0)),
            pl.BlockSpec((K, D), lambda b, t: (0, 0)),
            pl.BlockSpec((D, D), lambda b, t: (0, 0)),
        ],
        out_specs=pl.BlockSpec((1, TB, D), lambda b, t: (b, t, 0)),
        out_shape=jax.ShapeDtypeStruct((B, T, D), x.dtype),
        scratch_shapes=[pltpu.VMEM((NL, TB + 2 * HALO, 128), jnp.float32),
                        pltpu.VMEM((NL, TB, 128), jnp.float32),
                        pltpu.VMEM((D, 2 * D), jnp.bfloat16)],
        compiler_params=pltpu.CompilerParams(
            dimension_semantics=("arbitrary", "arbitrary"),
            vmem_limit_bytes=100 * 1024 * 1024,
        ),
    )(x, x, x, w_pw1, dw, w_pw2)
```

```python
import functools

import jax
import jax.numpy as jnp
import jax.experimental.pallas as pl
import jax.experimental.pallas.tpu as pltpu

_SIZES_16000 = (560, 1680, 4640, 9120)
_CH = 80
_HALO = 16


def _block_sizes(T):
    if T == sum(_SIZES_16000):
        return list(_SIZES_16000)
    for s in (2000, 1600, 800, 400, 160, 80):
        if T % s == 0:
            return [s] * (T // s)
    raise ValueError("unsupported sequence length")


@jax.jit
def pallas_standalone__conformer_conv_module__speech_kernel(x, w_pw1, dw, w_pw2):
    B, T, D = x.shape
    K = dw.shape[0]
    pad = K // 2
    CH, HALO = _CH, _HALO
    head = _block_sizes(T)
    assert pad <= 8 and D % 128 == 0
    assert all(s % CH == 0 and s % 16 == 0 and s > HALO for s in head)
    per_batch = [head[:] for _ in range(B)]
    per_batch[-1] = head[::-1] if B > 1 else head
    sizes = [s for pb in per_batch for s in pb]
    NB = len(sizes)
    starts = [sum(sizes[:i]) for i in range(NB)]
    firsts = [i for i in range(NB) if starts[i] % T == 0]
    lasts = [i for i in range(NB) if (starts[i] + sizes[i]) % T == 0]
    R = B * T
    L = CH // 8
    NL = D // 128
    MAXS = max(sizes)
    ustarts = [0] + [s + HALO for s in starts[1:]]
    usizes = [sizes[0] + HALO] + sizes[1:-1] + [sizes[-1] - HALO]

    def any_of(k, ks):
        return functools.reduce(jnp.logical_or, [k == kk for kk in ks])

    def kernel(x_hbm, w1_hbm, dw_hbm, w2_hbm, o_hbm, xall, oall, g_scr, s_scr, carry,
               w1_ref, dw_ref, w2_ref, w1h_scr, isem, osem, wsem):
        k = pl.program_id(0)
        r0 = jnp.int32(0)
        for kk in range(1, NB):
            r0 = jnp.where(k == kk, starts[kk], r0)
        first = any_of(k, firsts)
        last = any_of(k, lasts)

        def in_copy(start, size, kk):
            return pltpu.make_async_copy(
                x_hbm.at[pl.ds(start, size), :], xall.at[pl.ds(start, size), :], isem.at[kk])

        def out_copy(start, size, kk):
            return pltpu.make_async_copy(
                oall.at[pl.ds(start, size), :], o_hbm.at[pl.ds(start, size), :], osem.at[kk])

        wc = [pltpu.make_async_copy(w1_hbm, w1_ref, wsem.at[0]),
              pltpu.make_async_copy(dw_hbm, dw_ref, wsem.at[1]),
              pltpu.make_async_copy(w2_hbm, w2_ref, wsem.at[2])]

        @pl.when(k == 0)
        def _():
            wc[0].start()

        @pl.when(k < 1)
        def _():
            in_copy(ustarts[0], usizes[0], 0).start()
            wc[1].start()
            wc[2].start()

        @pl.when(k == 0)
        def _():
            in_copy(ustarts[1], usizes[1], 1).start()

        @pl.when(k < 1)
        def _():
            for kk in range(2, NB):
                in_copy(ustarts[kk], usizes[kk], kk).start()
            xall[R:R + HALO, :] = jnp.zeros((HALO, D), xall.dtype)
            wc[0].wait()
            w1h_scr[...] = w1_ref[...] * jnp.asarray(0.5, jnp.bfloat16)
            wc[1].wait()
            wc[2].wait()
            in_copy(ustarts[0], usizes[0], 0).wait()

        @pl.when(k == NB - 1)
        def _():
            in_copy(ustarts[NB - 1], usizes[NB - 1], NB - 1).wait()

        def compute(size):
            rr = pl.multiple_of(r0, 16)
            xs = xall[pl.ds(rr, size + HALO), :]
            h = jnp.dot(xs, w1h_scr[...], preferred_element_type=jnp.float32)
            a = h[:, :D]
            g = a + a * jnp.tanh(h[:, D:])
            for c in range(NL):
                gc = g[:, c * 128:(c + 1) * 128]
                g_scr[c, 0:8, :] = jnp.where(first, 0.0, carry[c])
                g_scr[c, 8:8 + size + HALO, :] = gc
                g_scr[c, 8 + size:16 + size, :] = jnp.where(last, 0.0, gc[size:size + 8])
                carry[c] = gc[size - 8:size]
            dwv = dw_ref[...].astype(jnp.float32) * 0.5
            o = 8 - pad
            wb = [[jnp.broadcast_to(dwv[kk:kk + 1, c * 128:(c + 1) * 128], (8, 128))
                   for kk in range(K)] for c in range(NL)]
            for q in range(size // CH):
                for c in range(NL):
                    def load(i):
                        return g_scr[c, pl.ds(q * CH + o + i, 8, stride=L), :]

                    win = [load(i) for i in range(K - 1)]
                    for j in range(L):
                        win.append(load(j + K - 1))
                        acc = win[0] * wb[c][0]
                        for kk in range(1, K):
                            acc = acc + win[kk] * wb[c][kk]
                        s_scr[c, pl.ds(q * CH + j, 8, stride=L), :] = acc + acc * jnp.tanh(acc)
                        win.pop(0)
            s = jnp.concatenate([s_scr[c, 0:size, :] for c in range(NL)], axis=1)
            oall[pl.ds(rr, size), :] = jnp.dot(
                s.astype(jnp.bfloat16), w2_ref[...],
                preferred_element_type=jnp.float32).astype(oall.dtype)
            out_copy(rr, size, k).start()

        for size in sorted(set(sizes)):
            ks = [kk for kk in range(NB) if sizes[kk] == size]
            mid = [kk for kk in ks if 0 < kk < NB - 1]
            if mid:
                @pl.when(any_of(k, mid))
                def _():
                    in_copy(pl.multiple_of(r0 + HALO, 16), size, k).wait()

            @pl.when(any_of(k, ks))
            def _():
                compute(size)

        @pl.when(k == NB - 1)
        def _():
            for kk in range(NB):
                out_copy(starts[kk], sizes[kk], kk).wait()

    out = pl.pallas_call(
        kernel,
        grid=(NB,),
        in_specs=[pl.BlockSpec(memory_space=pl.ANY)] * 4,
        out_specs=pl.BlockSpec(memory_space=pl.ANY),
        out_shape=jax.ShapeDtypeStruct((R, D), x.dtype),
        scratch_shapes=[
            pltpu.VMEM((R + HALO, D), jnp.bfloat16),
            pltpu.VMEM((R, D), jnp.bfloat16),
            pltpu.VMEM((NL, MAXS + 8 + HALO, 128), jnp.float32),
            pltpu.VMEM((NL, MAXS, 128), jnp.float32),
            pltpu.VMEM((NL, 8, 128), jnp.float32),
            pltpu.VMEM((D, 2 * D), jnp.bfloat16),
            pltpu.VMEM((K, D), jnp.bfloat16),
            pltpu.VMEM((D, D), jnp.bfloat16),
            pltpu.VMEM((D, 2 * D), jnp.bfloat16),
            pltpu.SemaphoreType.DMA((NB,)),
            pltpu.SemaphoreType.DMA((NB,)),
            pltpu.SemaphoreType.DMA((3,)),
        ],
        compiler_params=pltpu.CompilerParams(
            dimension_semantics=("arbitrary",),
            vmem_limit_bytes=110 * 1024 * 1024,
        ),
    )(x.reshape(R, D), w_pw1, dw, w_pw2)
    return out.reshape(B, T, D)
```

```python
import functools

import jax
import jax.numpy as jnp
import jax.experimental.pallas as pl
import jax.experimental.pallas.tpu as pltpu

_SIZES_16000 = (560, 1680, 4640, 9120)
_CH = 80
_HALO = 16


def _block_sizes(T):
    if T == sum(_SIZES_16000):
        return list(_SIZES_16000)
    for s in (2000, 1600, 800, 400, 160, 80):
        if T % s == 0:
            return [s] * (T // s)
    raise ValueError("unsupported sequence length")


@jax.jit
def pallas_standalone__conformer_conv_module__speech_kernel(x, w_pw1, dw, w_pw2):
    B, T, D = x.shape
    K = dw.shape[0]
    pad = K // 2
    CH, HALO = _CH, _HALO
    head = _block_sizes(T)
    assert pad <= 8 and D % 128 == 0
    assert all(s % CH == 0 and s % 16 == 0 and s > HALO for s in head)
    per_batch = [head[:] for _ in range(B)]
    per_batch[-1] = head[::-1] if B > 1 else head
    sizes = [s for pb in per_batch for s in pb]
    NB = len(sizes)
    starts = [sum(sizes[:i]) for i in range(NB)]
    firsts = [i for i in range(NB) if starts[i] % T == 0]
    lasts = [i for i in range(NB) if (starts[i] + sizes[i]) % T == 0]
    R = B * T
    L = CH // 8
    NL = D // 128
    MAXS = max(sizes)
    ustarts = [0] + [s + HALO for s in starts[1:]]
    usizes = [sizes[0] + HALO] + sizes[1:-1] + [sizes[-1] - HALO]

    def any_of(k, ks):
        return functools.reduce(jnp.logical_or, [k == kk for kk in ks])

    def kernel(x_hbm, w1_hbm, dw_hbm, w2_hbm, o_hbm, xall, oall, g_scr, s_scr, carry,
               w1_ref, dw_ref, w2_ref, w1h_scr, isem, osem, wsem):
        k = pl.program_id(0)
        r0 = jnp.int32(0)
        for kk in range(1, NB):
            r0 = jnp.where(k == kk, starts[kk], r0)
        first = any_of(k, firsts)
        last = any_of(k, lasts)

        def in_copy(start, size, kk):
            return pltpu.make_async_copy(
                x_hbm.at[pl.ds(start, size), :], xall.at[pl.ds(start, size), :], isem.at[kk])

        def out_copy(start, size, kk):
            return pltpu.make_async_copy(
                oall.at[pl.ds(start, size), :], o_hbm.at[pl.ds(start, size), :], osem.at[kk])

        wc = [pltpu.make_async_copy(w1_hbm, w1_ref, wsem.at[0]),
              pltpu.make_async_copy(dw_hbm, dw_ref, wsem.at[1]),
              pltpu.make_async_copy(w2_hbm, w2_ref, wsem.at[2])]

        @pl.when(k == 0)
        def _():
            wc[0].start()
            in_copy(ustarts[0], usizes[0], 0).start()
            wc[1].start()
            wc[2].start()
            xall[R:R + HALO, :] = jnp.zeros((HALO, D), xall.dtype)
            wc[0].wait()
            in_copy(ustarts[1], usizes[1], 1).start()
            w1h_scr[...] = w1_ref[...] * jnp.asarray(0.5, jnp.bfloat16)
            in_copy(ustarts[0], usizes[0], 0).wait()
            if NB > 2:
                in_copy(ustarts[2], usizes[2], 2).start()
            wc[1].wait()
            wc[2].wait()

        for kk in range(3, NB):
            @pl.when(k == kk - 2)
            def _():
                in_copy(ustarts[kk], usizes[kk], kk).start()

        @pl.when(k == NB - 1)
        def _():
            in_copy(ustarts[NB - 1], usizes[NB - 1], NB - 1).wait()

        def compute(size):
            rr = pl.multiple_of(r0, 16)
            xs = xall[pl.ds(rr, size + HALO), :]
            h = jnp.dot(xs, w1h_scr[...], preferred_element_type=jnp.float32)
            a = h[:, :D]
            g = a + a * jnp.tanh(h[:, D:])
            for c in range(NL):
                gc = g[:, c * 128:(c + 1) * 128]
                g_scr[c, 0:8, :] = jnp.where(first, 0.0, carry[c])
                g_scr[c, 8:8 + size + HALO, :] = gc
                g_scr[c, 8 + size:16 + size, :] = jnp.where(last, 0.0, gc[size:size + 8])
                carry[c] = gc[size - 8:size]
            dwv = dw_ref[...].astype(jnp.float32) * 0.5
            o = 8 - pad
            wb = [[jnp.broadcast_to(dwv[kk:kk + 1, c * 128:(c + 1) * 128], (8, 128))
                   for kk in range(K)] for c in range(NL)]
            for q in range(size // CH):
                for c in range(NL):
                    def load(i):
                        return g_scr[c, pl.ds(q * CH + o + i, 8, stride=L), :]

                    win = [load(i) for i in range(K - 1)]
                    for j in range(L):
                        win.append(load(j + K - 1))
                        acc = win[0] * wb[c][0]
                        for kk in range(1, K):
                            acc = acc + win[kk] * wb[c][kk]
                        s_scr[c, pl.ds(q * CH + j, 8, stride=L), :] = acc + acc * jnp.tanh(acc)
                        win.pop(0)
            s = jnp.concatenate([s_scr[c, 0:size, :] for c in range(NL)], axis=1)
            oall[pl.ds(rr, size), :] = jnp.dot(
                s.astype(jnp.bfloat16), w2_ref[...],
                preferred_element_type=jnp.float32).astype(oall.dtype)
            out_copy(rr, size, k).start()

        for size in sorted(set(sizes)):
            ks = [kk for kk in range(NB) if sizes[kk] == size]
            mid = [kk for kk in ks if 0 < kk < NB - 1]
            if mid:
                @pl.when(any_of(k, mid))
                def _():
                    in_copy(pl.multiple_of(r0 + HALO, 16), size, k).wait()

            @pl.when(any_of(k, ks))
            def _():
                compute(size)

        @pl.when(k == NB - 1)
        def _():
            for kk in range(NB):
                out_copy(starts[kk], sizes[kk], kk).wait()

    out = pl.pallas_call(
        kernel,
        grid=(NB,),
        in_specs=[pl.BlockSpec(memory_space=pl.ANY)] * 4,
        out_specs=pl.BlockSpec(memory_space=pl.ANY),
        out_shape=jax.ShapeDtypeStruct((R, D), x.dtype),
        scratch_shapes=[
            pltpu.VMEM((R + HALO, D), jnp.bfloat16),
            pltpu.VMEM((R, D), jnp.bfloat16),
            pltpu.VMEM((NL, MAXS + 8 + HALO, 128), jnp.float32),
            pltpu.VMEM((NL, MAXS, 128), jnp.float32),
            pltpu.VMEM((NL, 8, 128), jnp.float32),
            pltpu.VMEM((D, 2 * D), jnp.bfloat16),
            pltpu.VMEM((K, D), jnp.bfloat16),
            pltpu.VMEM((D, D), jnp.bfloat16),
            pltpu.VMEM((D, 2 * D), jnp.bfloat16),
            pltpu.SemaphoreType.DMA((NB,)),
            pltpu.SemaphoreType.DMA((NB,)),
            pltpu.SemaphoreType.DMA((3,)),
        ],
        compiler_params=pltpu.CompilerParams(
            dimension_semantics=("arbitrary",),
            vmem_limit_bytes=110 * 1024 * 1024,
        ),
    )(x.reshape(R, D), w_pw1, dw, w_pw2)
    return out.reshape(B, T, D)
```
